```python
import jax
import jax.numpy as jnp

def _softmax(x, axis=-1):
    return jax.nn.softmax(x, axis=axis)
def _gelu(x):
    return jax.nn.gelu(x, approximate=True)
def _silu(x):
    return jax.nn.silu(x)
def _sigmoid(x):
    return jax.nn.sigmoid(x)
def _layernorm(x, axis=-1, eps=1e-5):
    m = jnp.mean(x, axis=axis, keepdims=True)
    v = jnp.var(x, axis=axis, keepdims=True)
    return (x - m) / jnp.sqrt(v + eps)
def _scatter_add(tgt, idx, src, axis=0):
    return tgt.at[idx].add(src)
def _segment_sum(src, seg, n):
    return jax.ops.segment_sum(src, seg, n)
class _Rng:
    def __init__(self, key):
        self._k = key
    def _next(self):
        self._k, sub = jax.random.split(self._k)
        return sub
    def normal(self, shape):
        return jax.random.normal(self._next(), shape, dtype=jnp.bfloat16)
    def randint(self, lo, hi, shape):
        return jax.random.randint(self._next(), shape, lo, hi, dtype=jnp.int32)
    def uniform(self, shape, lo=0.0, hi=1.0):
        return jax.random.uniform(self._next(), shape, jnp.bfloat16, lo, hi)
    def permutation(self, n):
        return jax.random.permutation(self._next(), n)


kernel_name = 'interleave_layers__sliding_local_dilated__linear_kernel_hedgehog__prompt'

def setup_inputs():
    _rng = _Rng(jax.random.key(int.from_bytes(__import__("os").urandom(4), "little")))
    _w = (lambda a: (lambda t: t.astype(jnp.bfloat16) if jnp.issubdtype(t.dtype, jnp.floating) else t)(jnp.asarray(a)))
    def _A_setup():
        B, S, D = 1, 2048, 1024
        return {
            "x": _w((lambda *s: _rng.normal(s) * 0.05)(B, S, D)),
            "wqkv": _w((lambda *s: _rng.normal(s) * 0.05)(D, 3 * D)),
            "wo": _w((lambda *s: _rng.normal(s) * 0.05)(D, D)),
        }
    _A_in = _A_setup()

    def _B_setup():
        B, S, D, H = 1, 2048, 1024, 32
        Dh = D // H
        return {
            "x": _w((lambda *s: _rng.normal(s) * 0.05)(B, S, D)),
            "wqkv": _w((lambda *s: _rng.normal(s) * 0.05)(D, 3 * D)),
            "w_phi": _w((lambda *s: _rng.normal(s) * 0.05)(H, Dh, Dh) * (Dh ** -0.5)),
            "wo": _w((lambda *s: _rng.normal(s) * 0.05)(D, D)),
        }
    _B_in = _B_setup()

    return {
        "A_x": _A_in["x"],
        "A_wqkv": _A_in["wqkv"],
        "A_wo": _A_in["wo"],
        "B_x": _B_in["x"],
        "B_wqkv": _B_in["wqkv"],
        "B_w_phi": _B_in["w_phi"],
        "B_wo": _B_in["wo"],
    }

def reference(A_x, A_wqkv, A_wo, B_x, B_wqkv, B_w_phi, B_wo):
    def _A_ref(x, wqkv, wo):
        B, S, D = x.shape
        H = 32; Dh = D // H
        W, dil = 8, 2
        qkv = (lambda x, *d: x.transpose(*d))((x @ wqkv).reshape(B, S, 3, H, Dh), 2, 0, 3, 1, 4)
        q, k, v = qkv[0], qkv[1], qkv[2]
        scale = Dh ** -0.5
        pos = jnp.arange(S)
        off = jnp.arange(W) * dil
        idx = pos[:, None] - off[None, :]
        mask = idx >= 0
        idx_c = jnp.where(mask, idx, 0).reshape(-1)
        kg = k[:, :, idx_c, :].reshape(B, H, S, W, Dh)
        vg = v[:, :, idx_c, :].reshape(B, H, S, W, Dh)
        logits = jnp.einsum("bhsd,bhswd->bhsw", q, kg) * scale
        logits = jnp.where(mask[None, None, :, :], logits, -1e9)
        attn = _softmax(logits, axis=-1)
        o = jnp.einsum("bhsw,bhswd->bhsd", attn, vg)
        return (lambda x, *d: x.transpose(*d))(o, 0, 2, 1, 3).reshape(B, S, D) @ wo

    def _B_ref(x, wqkv, w_phi, wo):
        B, S, D = x.shape
        H = 32; Dh = D // H
        qkv = (lambda x, *d: x.transpose(*d))((x @ wqkv).reshape(B, S, 3, H, Dh), 2, 0, 3, 1, 4)
        q, k, v = qkv[0], qkv[1], qkv[2]
        pq = jnp.einsum("bhsd,hdf->bhsf", q, w_phi)
        pk = jnp.einsum("bhsd,hdf->bhsf", k, w_phi)
        phi_q = jnp.concatenate([_softmax(pq, axis=-1), _softmax(-pq, axis=-1)], axis=-1)
        phi_k = jnp.concatenate([_softmax(pk, axis=-1), _softmax(-pk, axis=-1)], axis=-1)
        kv = jnp.einsum("bhsf,bhsd->bhfd", phi_k, v)
        z  = jnp.einsum("bhsf->bhf", phi_k)
        num = jnp.einsum("bhqf,bhfd->bhqd", phi_q, kv)
        den = jnp.einsum("bhqf,bhf->bhq", phi_q, z)[..., None] + 1e-6
        o = num / den
        return (lambda x, *d: x.transpose(*d))(o, 0, 2, 1, 3).reshape(B, S, D) @ wo

    x = A_x
    x = x + _A_ref(_layernorm(x, axis=-1), A_wqkv, A_wo)
    x = x + _B_ref(_layernorm(x, axis=-1), B_wqkv, B_w_phi, B_wo)
    x = x + _A_ref(_layernorm(x, axis=-1), A_wqkv, A_wo)
    x = x + _B_ref(_layernorm(x, axis=-1), B_wqkv, B_w_phi, B_wo)
    return x
```

```python
import jax
import jax.numpy as jnp
import numpy as np
from jax import lax
from jax.experimental import pallas as pl
from jax.experimental.pallas import tpu as pltpu

S, D, H, DH = 2048, 1024, 32, 32
W = 8
HS = S // 2
NJ = HS // 128
GA = 256
GB = 128
F32, BF16 = jnp.float32, jnp.bfloat16
NT = (((1,), (1,)), ((), ()))


def _dot(a, b):
    return jnp.dot(a, b, preferred_element_type=F32)


def _dot_nt(a, b):
    return lax.dot_general(a, b, NT, preferred_element_type=F32)


def _iota(shape, dim):
    return lax.broadcasted_iota(jnp.int32, shape, dim)


def _kernel(x_hbm, aq_hbm, ao_hbm, bq_hbm, phi_hbm, bo_hbm, out_hbm,
            xb, xf, aq, ao, bq, bo, phi, aqT, aoT, bqT, boT,
            xT, xn, oT, buf0, buf1, pq, kv, zacc, sems):
    cps = [pltpu.make_async_copy(s, d, sems.at[i]) for i, (s, d) in enumerate(
        [(x_hbm, xb), (aq_hbm, aq), (ao_hbm, ao), (bq_hbm, bq), (phi_hbm, phi), (bo_hbm, bo)])]
    for c in cps:
        c.start()

    def ln_tile(v):
        mu = jnp.mean(v, axis=0, keepdims=True)
        c = v - mu
        var = jnp.mean(c * c, axis=0, keepdims=True)
        return (c * lax.rsqrt(var + 1e-5)).astype(BF16)

    cps[0].wait()

    @pl.loop(0, S // 256)
    def _(i):
        r = pl.multiple_of(i * 256, 256)
        for c in range(D // 128):
            xf[c, pl.ds(r, 256), :] = xb[pl.ds(r, 256), c * 128:(c + 1) * 128].astype(F32)

    def x_in(p):
        for j in range(NJ):
            v = jnp.concatenate(
                [xf[c, pl.ds(2 * j + p, 128, stride=16), :].T for c in range(D // 128)], axis=0)
            xT[p, :, j * 128:(j + 1) * 128] = v
            xn[p, :, j * 128:(j + 1) * 128] = ln_tile(v)

    x_in(0)
    x_in(1)

    r = _iota((GA, GA), 0)
    perm = jnp.where((r % 8) * DH + r // 8 == _iota((GA, GA), 1), 1.0, 0.0).astype(BF16)

    cps[1].wait()
    for sec in range(3):
        for g in range(D // GA):
            c0 = sec * D + g * GA
            aqT[g, sec * GA:(sec + 1) * GA, :] = _dot_nt(perm, aq[:, c0:c0 + GA]).astype(BF16)
    cps[2].wait()
    for g in range(D // GA):
        aoT[:, g * GA:(g + 1) * GA] = _dot(perm, ao[g * GA:(g + 1) * GA, :]).astype(BF16).T

    def prep_b():
        cps[3].wait()
        cps[4].wait()
        cps[5].wait()
        rr, cc = _iota((GB, GB), 0), _iota((GB, GB), 1)
        tile = jnp.where(_iota((DH, GB), 1) % DH == _iota((DH, GB), 0), 1.0, 0.0).astype(BF16)
        for g in range(D // GB):
            bd = jnp.where(rr // DH == cc // DH, _dot(phi[g * GB:(g + 1) * GB, :], tile), 0.0)
            bdT = bd.T.astype(BF16)
            for sec in range(2):
                c0 = sec * D + g * GB
                bqT[g, sec * GB:(sec + 1) * GB, :] = _dot_nt(bdT, bq[:, c0:c0 + GB]).astype(BF16)
            bqT[g, 2 * GB:, :] = bq[:, 2 * D + g * GB:2 * D + (g + 1) * GB].T
            boT[:, g * GB:(g + 1) * GB] = bo[g * GB:(g + 1) * GB, :].T

    def out_proj(wT):
        CH = 512

        @pl.loop(0, S // CH)
        def _(i):
            p = i // (HS // CH)
            c = pl.multiple_of((i % (HS // CH)) * CH, CH)
            y = xT[p, :, pl.ds(c, CH)] + _dot(wT[...], oT[p, :, pl.ds(c, CH)])
            xT[p, :, pl.ds(c, CH)] = y
            xn[p, :, pl.ds(c, CH)] = ln_tile(y)

    def a_mm(u, buf):
        y = _dot(aqT[u // 2], xn[u % 2])
        buf[0:3 * GA, :] = y
        buf[3 * GA:, 128:] = pltpu.roll(y[GA:, 128:].reshape(2 * GA, NJ - 1, 128), 1, 2).reshape(2 * GA, HS - 128)

    def a_att(u, buf):
        r0 = pl.multiple_of((u // 2) * GA, GA)
        lane = _iota((8, 128), 1)
        for j in range(NJ):
            def src(sec, w):
                if j >= w:
                    v = buf[sec * GA:(sec + 1) * GA, (j - w) * 128:(j - w + 1) * 128]
                else:
                    jj = j - w + NJ
                    v = buf[(sec + 2) * GA:(sec + 3) * GA, jj * 128:(jj + 1) * 128]
                return v.reshape(DH, 8, 128)
            q = src(0, 0)
            lg = []
            for w in range(W):
                l = jnp.sum(q * src(1, w), axis=0) * (DH ** -0.5)
                if j < w:
                    l = jnp.where(lane == 0, -1e9, l)
                lg.append(l)
            m = lg[0]
            for l in lg[1:]:
                m = jnp.maximum(m, l)
            e = [jnp.exp(l - m) for l in lg]
            den = e[0]
            for t in e[1:]:
                den = den + t
            inv = 1.0 / den
            o = (e[0] * inv) * src(2, 0)
            for w in range(1, W):
                o = o + (e[w] * inv) * src(2, w)
            oT[u % 2, pl.ds(r0, GA), j * 128:(j + 1) * 128] = o.reshape(GA, 128).astype(BF16)

    def layer_a():
        n = 2 * (D // GA)
        a_mm(0, buf0)

        @pl.loop(0, n // 2 - 1)
        def _(i):
            a_mm(2 * i + 1, buf1)
            a_att(2 * i, buf0)
            a_mm(2 * i + 2, buf0)
            a_att(2 * i + 1, buf1)

        a_mm(n - 1, buf1)
        a_att(n - 2, buf0)
        a_att(n - 1, buf1)
        out_proj(aoT)

    def feat(y):
        outs = []
        for h in range(GB // DH):
            t = y[h * DH:(h + 1) * DH]
            ep = jnp.exp(t - jnp.max(t, axis=0, keepdims=True))
            en = jnp.exp(jnp.min(t, axis=0, keepdims=True) - t)
            outs.append(ep * (1.0 / jnp.sum(ep, axis=0, keepdims=True)))
            outs.append(en * (1.0 / jnp.sum(en, axis=0, keepdims=True)))
        return outs

    def layer_b():
        @pl.loop(0, D // GB)
        def _(g):
            r0 = pl.multiple_of(g * 2 * GB, 2 * GB)
            acc = None
            z = None
            for p in range(2):
                y = _dot(bqT[g], xn[p])
                pq[p, pl.ds(r0, 2 * GB), :] = jnp.concatenate(feat(y[:GB]), axis=0).astype(BF16)
                fk = jnp.concatenate(feat(y[GB:2 * GB]), axis=0)
                t = _dot_nt(y[2 * GB:].astype(BF16), fk.astype(BF16))
                acc = t if acc is None else acc + t
                for j in range(NJ):
                    s = fk[:, j * 128:(j + 1) * 128]
                    z = s if z is None else z + s
            rr, cc = _iota((GB, 2 * GB), 0), _iota((GB, 2 * GB), 1)
            kv[g, 0:GB, :] = jnp.where(rr // DH == cc // (2 * DH), acc, 0.0).astype(BF16)
            zr = jnp.sum(z.T, axis=0, keepdims=True)
            rr, cc = _iota((16, 2 * GB), 0), _iota((16, 2 * GB), 1)
            kv[g, GB:, :] = jnp.where(rr == cc // (2 * DH), zr, 0.0).astype(BF16)

        @pl.loop(0, D // GB)
        def _(g):
            r0 = pl.multiple_of(g * 2 * GB, 2 * GB)
            r1 = pl.multiple_of(g * GB, GB)
            for p in range(2):
                t = _dot(kv[g], pq[p, pl.ds(r0, 2 * GB), :])
                inv = 1.0 / (t[GB:GB + 8] + 1e-6)
                o = jnp.concatenate(
                    [t[h * DH:(h + 1) * DH] * inv[h:h + 1] for h in range(GB // DH)], axis=0)
                oT[p, pl.ds(r1, GB), :] = o.astype(BF16)

        out_proj(boT)

    prep_b()

    @pl.loop(0, 2)
    def _(_):
        layer_a()
        layer_b()

    for p in range(2):
        for j in range(NJ):
            for c in range(D // 128):
                xf[c, pl.ds(2 * j + p, 128, stride=16), :] = xT[
                    p, c * 128:(c + 1) * 128, j * 128:(j + 1) * 128].T

    @pl.loop(0, S // 256)
    def _(i):
        r = pl.multiple_of(i * 256, 256)
        for c in range(D // 128):
            xb[pl.ds(r, 256), c * 128:(c + 1) * 128] = xf[c, pl.ds(r, 256), :].astype(BF16)

    cp = pltpu.make_async_copy(xb, out_hbm, sems.at[0])
    cp.start()
    cp.wait()


@jax.jit
def pallas_interleave_layers__sliding_local_dilated__linear_kernel_hedgehog__prompt_kernel(
    A_x, A_wqkv, A_wo, B_x, B_wqkv, B_w_phi, B_wo,
):
    del B_x
    vm = pltpu.VMEM
    out = pl.pallas_call(
        _kernel,
        out_shape=jax.ShapeDtypeStruct((S, D), BF16),
        in_specs=[pl.BlockSpec(memory_space=pl.ANY)] * 6,
        out_specs=pl.BlockSpec(memory_space=pl.ANY),
        scratch_shapes=[
            vm((S, D), BF16), vm((D // 128, S, 128), F32),
            vm((D, 3 * D), BF16), vm((D, D), BF16), vm((D, 3 * D), BF16), vm((D, D), BF16),
            vm((D, DH), BF16),
            vm((D // GA, 3 * GA, D), BF16), vm((D, D), BF16),
            vm((D // GB, 3 * GB, D), BF16), vm((D, D), BF16),
            vm((2, D, HS), F32), vm((2, D, HS), BF16), vm((2, D, HS), BF16),
            vm((5 * GA, HS), F32), vm((5 * GA, HS), F32),
            vm((2, 2 * D, HS), BF16), vm((D // GB, GB + 16, 2 * GB), BF16),
            vm((8, 128), F32),
            pltpu.SemaphoreType.DMA((6,)),
        ],
        compiler_params=pltpu.CompilerParams(vmem_limit_bytes=120 * 1024 * 1024),
    )(A_x.reshape(S, D), A_wqkv, A_wo, B_wqkv, B_w_phi.reshape(D, DH), B_wo)
    return out.reshape(1, S, D)
```

```python
import functools

import jax
import jax.numpy as jnp
from jax import lax
from jax.experimental import pallas as pl
from jax.experimental.pallas import tpu as pltpu

S, D, H, DH = 2048, 1024, 32, 32
W = 8
HS = S // 2
NJ = HS // 128
GA = 256
GB = 128
F32, BF16, U32 = jnp.float32, jnp.bfloat16, jnp.uint32
NT = (((1,), (1,)), ((), ()))


def _dot(a, b):
    return jnp.dot(a, b, preferred_element_type=F32)


def _dot_nt(a, b):
    return lax.dot_general(a, b, NT, preferred_element_type=F32)


def _iota(shape, dim):
    return lax.broadcasted_iota(jnp.int32, shape, dim)


def _ld(v):
    return pltpu.bitcast(v, BF16)


def _st(v):
    return pltpu.bitcast(v.astype(BF16), U32)


def _top(v):
    return pltpu.bitcast(v.astype(BF16).astype(F32), U32)


def _kernel(x_hbm, aq_hbm, ao_hbm, bq_hbm, phi_hbm, bo_hbm, out_hbm,
            xb0, xb1, xb2, xb3, xu0, xu1, aq0, aq1, aq2, aq3, ao, bq, bo, phi,
            aqT, aoT, bqT, boT, xT0, xT1, xn0, xn1, oT0, oT1, buf0, buf1, pq0, pq1, kv, sems):
    xb, xu, aq = (xb0, xb1, xb2, xb3), (xu0, xu1), (aq0, aq1, aq2, aq3)
    xT, xn, oT, buf, pq = (xT0, xT1), (xn0, xn1), (oT0, oT1), (buf0, buf1), (pq0, pq1)
    NC = D // GA
    cols = lambda c: pl.ds(c * GA, GA)
    tile = lambda j: slice(j * 128, (j + 1) * 128)
    pairs = [(x_hbm.at[:, cols(c)], xb[c]) for c in range(NC)]
    pairs += [(aq_hbm.at[:, cols(sec * NC + g)], aq[g].at[sec]) for g in range(NC) for sec in range(3)]
    pairs += [(ao_hbm, ao), (bq_hbm, bq), (phi_hbm, phi), (bo_hbm, bo)]
    cps = [pltpu.make_async_copy(s, d, sems.at[i]) for i, (s, d) in enumerate(pairs)]
    for c in cps[:7]:
        c.start()

    def set_x(p, rows, y):
        xT[p][rows, :] = y

    def ln(p):
        for j in range(NJ):
            v = xT[p][:, tile(j)]
            c = v - jnp.mean(v, axis=0, keepdims=True)
            var = jnp.mean(c * c, axis=0, keepdims=True)
            xn[p][:, tile(j)] = _st(c * lax.rsqrt(var + 1e-5))

    for c in range(NC):
        cps[c].wait()
        if c == 0:
            for cp in cps[7:]:
                cp.start()
        for t in range(2):
            xu[t][...] = pltpu.bitcast(xb[c][:, tile(t)], U32)
            rows = slice(c * GA + t * 128, c * GA + (t + 1) * 128)
            for j in range(NJ):
                v = xu[t][pl.ds(j, 128, stride=NJ), :].T
                xT0[rows, tile(j)] = pltpu.bitcast(v << 16, F32)
                xT1[rows, tile(j)] = pltpu.bitcast(v & jnp.uint32(0xFFFF0000), F32)

    r, cc = _iota((128, 128), 0), _iota((128, 128), 1)
    perm = [jnp.where((r % 4) * DH + ((r // 4) ^ b) == cc, 1.0, 0.0).astype(BF16) for b in range(2)]

    def prep_aq(g):
        for sec in range(3):
            cps[NC + 3 * g + sec].wait()
            a, b = (_dot_nt(perm[t], aq[g][sec, :, tile(t)]).reshape(16, 8, D) for t in range(2))
            lo = _iota((16, 8, D), 1) < 4
            o = jnp.stack([jnp.where(lo, a, b), pltpu.roll(jnp.where(lo, b, a), 4, 1)], axis=1)
            aqT[g, sec * 128:(sec + 1) * 128, :] = _st(o.reshape(GA, D))

    def prep_ao():
        cps[-4].wait()
        r = _iota((GA, GA), 0)
        pm = jnp.where((r % 8) * DH + r // 8 == _iota((GA, GA), 1), 1.0, 0.0).astype(BF16)
        for g in range(NC):
            t = _dot(pm, ao[g * GA:(g + 1) * GA, :]).astype(BF16).T
            aoT[:, g * GA:(g + 1) * GA] = pltpu.bitcast(t, U32)

    def prep_b():
        for cp in cps[-3:]:
            cp.wait()
        rep = jnp.where(_iota((DH, GB), 1) % DH == _iota((DH, GB), 0), 1.0, 0.0).astype(BF16)
        for g in range(D // GB):
            bd = jnp.where(r // DH == cc // DH, _dot(phi[tile(g), :], rep), 0.0)
            bdT = bd.T.astype(BF16)
            for sec in range(2):
                bqT[g, sec * 64:(sec + 1) * 64, :] = _st(_dot_nt(bdT, bq[:, tile(sec * 8 + g)]))
            bqT[g, 128:, :] = pltpu.bitcast(bq[:, tile(16 + g)].T, U32)
            boT[:, tile(g)] = pltpu.bitcast(bo[tile(g), :].T, U32)

    def out_proj(wT, p):
        xT[p][...] += _dot(_ld(wT[...]), _ld(oT[p][...]))

    def a_mm(p, g):
        b = buf[g % 2]
        y = _dot(_ld(aqT[g]), _ld(xn[p][...]))
        b[0:3 * GA, :] = y
        for j in range(1, NJ):
            b[3 * GA:, tile(j)] = pltpu.roll(y[GA:, tile(j)], 1, 1)

    def a_att(p, g):
        b = buf[g % 2]
        lane = _iota((8, 128), 1)
        for j in range(NJ):
            def src(sec, w):
                sec = sec if j >= w else sec + 2
                return b[sec * GA:(sec + 1) * GA, tile((j - w) % NJ)].reshape(DH, 8, 128)
            q = src(0, 0)
            lg = []
            for w in range(W):
                l = jnp.sum(q * src(1, w), axis=0) * (DH ** -0.5)
                if j < w:
                    l = jnp.where(lane == 0, -1e9, l)
                lg.append(l)
            m = functools.reduce(jnp.maximum, lg)
            e = [jnp.exp(l - m) for l in lg]
            inv = 1.0 / sum(e[1:], e[0])
            o = (e[0] * inv) * src(2, 0)
            for w in range(1, W):
                o = o + (e[w] * inv) * src(2, w)
            oT[p][g * 128:(g + 1) * 128, tile(j)] = _st(o.reshape(GA, 128))

    def layer_a(first):
        us = [(p, g) for p in range(2) for g in range(NC)]
        if first:
            ln(0)
            prep_aq(0)
        else:
            ln(1)
        a_mm(*us[0])
        for i in range(1, len(us)):
            if first and i < NC:
                prep_aq(i)
            if first and i == 1:
                ln(1)
            a_mm(*us[i])
            a_att(*us[i - 1])
            if first and i == 3:
                prep_ao()
            if first and i == 5:
                prep_b()
        a_att(*us[-1])
        out_proj(aoT, 0)
        ln(0)
        out_proj(aoT, 1)

    def feat(y):
        outs = []
        for h in range(GB // DH):
            t = y[h * DH:(h + 1) * DH]
            ep = jnp.exp(t - jnp.max(t, axis=0, keepdims=True))
            en = jnp.exp(jnp.min(t, axis=0, keepdims=True) - t)
            outs.append(ep * (1.0 / jnp.sum(ep, axis=0, keepdims=True)))
            outs.append(en * (1.0 / jnp.sum(en, axis=0, keepdims=True)))
        return jnp.concatenate(outs, axis=0)

    def b_qkv(p, g):
        y = _dot(_ld(bqT[g]), _ld(xn[p][...]))
        pq[p][tile(g), :] = _st(feat(y[:GB]))
        fk = feat(y[GB:2 * GB]).astype(BF16)
        ones = jnp.ones((16, HS), BF16)
        for t in range(2):
            v = y[2 * GB + t * 64:2 * GB + (t + 1) * 64].astype(BF16)
            a = _dot_nt(jnp.concatenate([v, ones], axis=0), fk[tile(t)])
            if p == 0:
                kv[2 * g + t] = a
            else:
                rr = _iota((80, 128), 0)
                hd = jnp.where(rr < 64, rr // DH, rr - 64)
                kv[2 * g + t] = jnp.where(hd == _iota((80, 128), 1) // 64, a + kv[2 * g + t], 0.0)

    def b_out(p):
        for t in range(H // 2):
            y = _dot(kv[t].astype(BF16), _ld(pq[p][t * 64:(t + 1) * 64, :]))
            inv = 1.0 / (y[64:72] + 1e-6)
            o = jnp.concatenate([y[h * DH:(h + 1) * DH] * inv[h:h + 1] for h in range(2)], axis=0)
            oT[p][t * DH:(t + 1) * DH, :] = _st(o)

    def finish():
        cps = []
        for c in range(NC):
            rows = slice(c * GA, (c + 1) * GA)
            w = _ld(boT[tile(c), :])
            y0, y1 = (xT[p][rows, :] + _dot(w, _ld(oT[p][...])) for p in range(2))
            u = (_top(y0) >> 16) | _top(y1)
            for t in range(2):
                for j in range(NJ):
                    xu[t][pl.ds(j, 128, stride=NJ), :] = u[tile(t), tile(j)].T
                xb[c][:, tile(t)] = _ld(xu[t][...])
            cps.append(pltpu.make_async_copy(xb[c], out_hbm.at[:, cols(c)], sems.at[c]))
            cps[-1].start()
        for cp in cps:
            cp.wait()

    def layer_b(last):
        ln(1)
        for p in range(2):
            for g in range(D // GB):
                b_qkv(p, g)
        b_out(0)
        b_out(1)
        if last:
            finish()
        else:
            out_proj(boT, 0)
            ln(0)
            out_proj(boT, 1)

    for l in range(2):
        layer_a(l == 0)
        layer_b(l == 1)


@jax.jit
def pallas_interleave_layers__sliding_local_dilated__linear_kernel_hedgehog__prompt_kernel(
    A_x, A_wqkv, A_wo, B_x, B_wqkv, B_w_phi, B_wo,
):
    del B_x
    vm = pltpu.VMEM
    out = pl.pallas_call(
        _kernel,
        out_shape=jax.ShapeDtypeStruct((S, D), BF16),
        in_specs=[pl.BlockSpec(memory_space=pl.ANY)] * 6,
        out_specs=pl.BlockSpec(memory_space=pl.ANY),
        scratch_shapes=[
            *[vm((S, GA), BF16)] * 4, *[vm((HS, 128), U32)] * 2, *[vm((3, D, GA), BF16)] * 4,
            vm((D, D), BF16), vm((D, 3 * D), BF16), vm((D, D), BF16), vm((D, DH), BF16),
            vm((D // GA, 3 * GA // 2, D), U32), vm((D // 2, D), U32),
            vm((D // GB, 3 * GB // 2, D), U32), vm((D // 2, D), U32),
            *[vm((D, HS), F32)] * 2, *[vm((D // 2, HS), U32)] * 4,
            *[vm((5 * GA, HS), F32)] * 2, *[vm((D, HS), U32)] * 2,
            vm((H // 2, 80, 128), F32),
            pltpu.SemaphoreType.DMA((20,)),
        ],
        compiler_params=pltpu.CompilerParams(vmem_limit_bytes=120 * 1024 * 1024),
    )(A_x.reshape(S, D), A_wqkv, A_wo, B_wqkv, B_w_phi.reshape(D, DH), B_wo)
    return out.reshape(1, S, D)
```

```python
import functools

import jax
import jax.numpy as jnp
from jax import lax
from jax.experimental import pallas as pl
from jax.experimental.pallas import tpu as pltpu

S, D, H, DH = 2048, 1024, 32, 32
W = 8
HS = S // 2
NJ = HS // 128
GA = 256
GB = 128
F32, BF16, U32 = jnp.float32, jnp.bfloat16, jnp.uint32
NT = (((1,), (1,)), ((), ()))


def _dot(a, b):
    return jnp.dot(a, b, preferred_element_type=F32)


def _dot_nt(a, b):
    return lax.dot_general(a, b, NT, preferred_element_type=F32)


def _iota(shape, dim):
    return lax.broadcasted_iota(jnp.int32, shape, dim)


def _ld(v):
    return pltpu.bitcast(v, BF16)


def _st(v):
    return pltpu.bitcast(v.astype(BF16), U32)


def _top(v):
    return pltpu.bitcast(v.astype(BF16).astype(F32), U32)


def _kernel(x_hbm, aq_hbm, ao_hbm, bq_hbm, phi_hbm, bo_hbm, out_hbm,
            xb0, xb1, xb2, xb3, xu0, xu1, aq0, aq1, aq2, aq3, ao, bq, bo, phi,
            aqT, aoT, bqT, boT, xT0, xT1, xn0, xn1, oT0, oT1, buf0, buf1, pq0, pq1, kv, sems):
    xb, xu, aq = (xb0, xb1, xb2, xb3), (xu0, xu1), (aq0, aq1, aq2, aq3)
    xT, xn, oT, buf, pq = (xT0, xT1), (xn0, xn1), (oT0, oT1), (buf0, buf1), (pq0, pq1)
    NC = D // GA
    cols = lambda c: pl.ds(c * GA, GA)
    tile = lambda j: slice(j * 128, (j + 1) * 128)
    pairs = [(x_hbm.at[:, cols(c)], xb[c]) for c in range(NC)]
    pairs += [(aq_hbm.at[:, cols(sec * NC + g)], aq[g].at[sec]) for g in range(NC) for sec in range(3)]
    pairs += [(ao_hbm, ao), (bq_hbm, bq), (phi_hbm, phi), (bo_hbm, bo)]
    cps = [pltpu.make_async_copy(s, d, sems.at[i]) for i, (s, d) in enumerate(pairs)]
    for c in cps[:7]:
        c.start()

    def set_x(p, rows, y):
        xT[p][rows, :] = y

    def run(*gens):
        for _ in zip(*gens):
            pass

    def ln(p):
        for j in range(NJ):
            v = xT[p][:, tile(j)]
            c = v - jnp.mean(v, axis=0, keepdims=True)
            var = jnp.mean(c * c, axis=0, keepdims=True)
            xn[p][:, tile(j)] = _st(c * lax.rsqrt(var + 1e-5))
            yield

    for c in range(NC):
        cps[c].wait()
        if c == 0:
            for cp in cps[7:]:
                cp.start()
        for t in range(2):
            xu[t][...] = pltpu.bitcast(xb[c][:, tile(t)], U32)
            rows = slice(c * GA + t * 128, c * GA + (t + 1) * 128)
            for j in range(NJ):
                v = xu[t][pl.ds(j, 128, stride=NJ), :].T
                xT0[rows, tile(j)] = pltpu.bitcast(v << 16, F32)
                xT1[rows, tile(j)] = pltpu.bitcast(v & jnp.uint32(0xFFFF0000), F32)

    r, cc = _iota((128, 128), 0), _iota((128, 128), 1)
    perm = [jnp.where((r % 4) * DH + ((r // 4) ^ b) == cc, 1.0, 0.0).astype(BF16) for b in range(2)]

    def merge(a, b):
        a, b = a.reshape(16, 8, D), b.reshape(16, 8, D)
        lo = _iota((16, 8, D), 1) < 4
        o = jnp.stack([jnp.where(lo, a, b), pltpu.roll(jnp.where(lo, b, a), 4, 1)], axis=1)
        return o.reshape(GA, D)

    def prep_aq(g):
        for sec in range(3):
            cps[NC + 3 * g + sec].wait()
        for sec in range(3):
            a, b = (_dot_nt(perm[t], aq[g][sec, :, tile(t)]) for t in range(2))
            aqT[g, tile(sec), :] = _st(merge(a, b))

    def prep_ao():
        for cp in cps[-4:]:
            cp.wait()
        for g in range(NC):
            a, b = (_dot(perm[t], ao[tile(2 * g + t), :]) for t in range(2))
            aoT[:, g * GA:(g + 1) * GA] = pltpu.bitcast(merge(a, b).astype(BF16).T, U32)

    def prep_b():
        rep = jnp.where(_iota((DH, GB), 1) % DH == _iota((DH, GB), 0), 1.0, 0.0).astype(BF16)
        for g in range(D // GB):
            bd = jnp.where(r // DH == cc // DH, _dot(phi[tile(g), :], rep), 0.0)
            bdT = bd.T.astype(BF16)
            for sec in range(2):
                bqT[g, sec * 64:(sec + 1) * 64, :] = _st(_dot_nt(bdT, bq[:, tile(sec * 8 + g)]))
            bqT[g, 128:, :] = pltpu.bitcast(bq[:, tile(16 + g)].T, U32)
            boT[:, tile(g)] = pltpu.bitcast(bo[tile(g), :].T, U32)

    def out_proj(wT, p):
        for j in range(NJ):
            xT[p][:, tile(j)] += _dot(_ld(wT[...]), _ld(oT[p][:, tile(j)]))
            yield

    def a_mm(p, g):
        b = buf[g % 2]
        for j in range(NJ):
            y = _dot(_ld(aqT[g]), _ld(xn[p][:, tile(j)]))
            b[0:3 * GA, tile(j)] = y
            if j:
                b[3 * GA:, tile(j)] = pltpu.roll(y[GA:], 1, 1)
            yield

    def a_att(p, g):
        b = buf[g % 2]
        lane = _iota((8, 128), 1)
        for j in range(NJ):
            def src(sec, w):
                sec = sec if j >= w else sec + 2
                return b[sec * GA:(sec + 1) * GA, tile((j - w) % NJ)].reshape(DH, 8, 128)
            q = src(0, 0)
            lg = []
            for w in range(W):
                l = jnp.sum(q * src(1, w), axis=0) * (DH ** -0.5)
                if j < w:
                    l = jnp.where(lane == 0, -1e9, l)
                lg.append(l)
            m = functools.reduce(jnp.maximum, lg)
            e = [jnp.exp(l - m) for l in lg]
            inv = 1.0 / sum(e[1:], e[0])
            o = (e[0] * inv) * src(2, 0)
            for w in range(1, W):
                o = o + (e[w] * inv) * src(2, w)
            oT[p][g * 128:(g + 1) * 128, tile(j)] = _st(o.reshape(GA, 128))
            yield

    def layer_a(first):
        us = [(p, g) for p in range(2) for g in range(NC)]
        if first:
            prep_aq(0)
            run(ln(0), a_mm(*us[0]), ln(1))
        else:
            run(ln(1), a_mm(*us[0]))
        for i in range(1, len(us)):
            if first and i < NC:
                prep_aq(i)
            if first and i == 5:
                prep_ao()
                prep_b()
            run(a_mm(*us[i]), a_att(*us[i - 1]))
        run(out_proj(aoT, 0), a_att(*us[-1]))
        run(out_proj(aoT, 1), ln(0))

    def feat(y):
        outs = []
        for h in range(GB // DH):
            t = y[h * DH:(h + 1) * DH]
            ep = jnp.exp(t - jnp.max(t, axis=0, keepdims=True))
            en = jnp.exp(jnp.min(t, axis=0, keepdims=True) - t)
            outs.append(ep * (1.0 / jnp.sum(ep, axis=0, keepdims=True)))
            outs.append(en * (1.0 / jnp.sum(en, axis=0, keepdims=True)))
        return jnp.concatenate(outs, axis=0)

    def b_qkv(p, g):
        y = _dot(_ld(bqT[g]), _ld(xn[p][...]))
        pq[p][tile(g), :] = _st(feat(y[:GB]))
        fk = feat(y[GB:2 * GB]).astype(BF16)
        ones = jnp.ones((16, HS), BF16)
        for t in range(2):
            v = y[2 * GB + t * 64:2 * GB + (t + 1) * 64].astype(BF16)
            a = _dot_nt(jnp.concatenate([v, ones], axis=0), fk[tile(t)])
            if p == 0:
                kv[2 * g + t] = a
            else:
                rr = _iota((80, 128), 0)
                hd = jnp.where(rr < 64, rr // DH, rr - 64)
                kv[2 * g + t] = jnp.where(hd == _iota((80, 128), 1) // 64, a + kv[2 * g + t], 0.0)

    def b_out(p):
        for t in range(H // 2):
            y = _dot(kv[t].astype(BF16), _ld(pq[p][t * 64:(t + 1) * 64, :]))
            inv = 1.0 / (y[64:72] + 1e-6)
            o = jnp.concatenate([y[h * DH:(h + 1) * DH] * inv[h:h + 1] for h in range(2)], axis=0)
            oT[p][t * DH:(t + 1) * DH, :] = _st(o)

    def finish():
        cps = []
        for c in range(NC):
            rows = slice(c * GA, (c + 1) * GA)
            w = _ld(boT[tile(c), :])
            y0, y1 = (xT[p][rows, :] + _dot(w, _ld(oT[p][...])) for p in range(2))
            u = (_top(y0) >> 16) | _top(y1)
            for t in range(2):
                for j in range(NJ):
                    xu[t][pl.ds(j, 128, stride=NJ), :] = u[tile(t), tile(j)].T
                xb[c][:, tile(t)] = _ld(xu[t][...])
            cps.append(pltpu.make_async_copy(xb[c], out_hbm.at[:, cols(c)], sems.at[c]))
            cps[-1].start()
        for cp in cps:
            cp.wait()

    def layer_b(last):
        run(ln(1))
        for p in range(2):
            for g in range(D // GB):
                b_qkv(p, g)
        b_out(0)
        b_out(1)
        if last:
            finish()
        else:
            run(out_proj(boT, 0))
            run(out_proj(boT, 1), ln(0))

    for l in range(2):
        layer_a(l == 0)
        layer_b(l == 1)


@jax.jit
def pallas_interleave_layers__sliding_local_dilated__linear_kernel_hedgehog__prompt_kernel(
    A_x, A_wqkv, A_wo, B_x, B_wqkv, B_w_phi, B_wo,
):
    del B_x
    vm = pltpu.VMEM
    out = pl.pallas_call(
        _kernel,
        out_shape=jax.ShapeDtypeStruct((S, D), BF16),
        in_specs=[pl.BlockSpec(memory_space=pl.ANY)] * 6,
        out_specs=pl.BlockSpec(memory_space=pl.ANY),
        scratch_shapes=[
            *[vm((S, GA), BF16)] * 4, *[vm((HS, 128), U32)] * 2, *[vm((3, D, GA), BF16)] * 4,
            vm((D, D), BF16), vm((D, 3 * D), BF16), vm((D, D), BF16), vm((D, DH), BF16),
            vm((D // GA, 3 * GA // 2, D), U32), vm((D // 2, D), U32),
            vm((D // GB, 3 * GB // 2, D), U32), vm((D // 2, D), U32),
            *[vm((D, HS), F32)] * 2, *[vm((D // 2, HS), U32)] * 4,
            *[vm((5 * GA, HS), F32)] * 2, *[vm((D, HS), U32)] * 2,
            vm((H // 2, 80, 128), F32),
            pltpu.SemaphoreType.DMA((20,)),
        ],
        compiler_params=pltpu.CompilerParams(vmem_limit_bytes=120 * 1024 * 1024),
    )(A_x.reshape(S, D), A_wqkv, A_wo, B_wqkv, B_w_phi.reshape(D, DH), B_wo)
    return out.reshape(1, S, D)
```

```python
import functools

import jax
import jax.numpy as jnp
from jax import lax
from jax.experimental import pallas as pl
from jax.experimental.pallas import tpu as pltpu

S, D, H, DH = 2048, 1024, 32, 32
W = 8
CD = 8
HS = S // 2
NJ = HS // 128
GA = 256
GB = 128
F32, BF16, U32 = jnp.float32, jnp.bfloat16, jnp.uint32
NT = (((1,), (1,)), ((), ()))


def _dot(a, b):
    return jnp.dot(a, b, preferred_element_type=F32)


def _dot_nt(a, b):
    return lax.dot_general(a, b, NT, preferred_element_type=F32)


def _iota(shape, dim):
    return lax.broadcasted_iota(jnp.int32, shape, dim)


def _ld(v):
    return pltpu.bitcast(v, BF16)


def _st(v):
    return pltpu.bitcast(v.astype(BF16), U32)


def _top(v):
    return pltpu.bitcast(v.astype(BF16).astype(F32), U32)


def _kernel(x_hbm, aq_hbm, ao_hbm, bq_hbm, phi_hbm, bo_hbm, out_hbm,
            xb0, xb1, xb2, xb3, xu0, xu1, aq0, aq1, aq2, aq3, ao, bq, bo, phi,
            aqT, aoT, bqT, boT, xT0, xT1, xnn, oTT, buf0, buf1, pq0, pq1, kv, sems):
    xb, xu, aq = (xb0, xb1, xb2, xb3), (xu0, xu1), (aq0, aq1, aq2, aq3)
    xT, xn, oT, buf, pq = (xT0, xT1), (xnn.at[0], xnn.at[1]), (oTT.at[0], oTT.at[1]), (buf0, buf1), (pq0, pq1)
    NC = D // GA
    cols = lambda c: pl.ds(c * GA, GA)
    tile = lambda j: slice(j * 128, (j + 1) * 128)
    pairs = [(x_hbm.at[:, cols(c)], xb[c]) for c in range(NC)]
    pairs += [(aq_hbm.at[:, cols(sec * NC + g)], aq[g].at[sec]) for g in range(NC) for sec in range(3)]
    pairs += [(ao_hbm, ao), (bq_hbm, bq), (phi_hbm, phi), (bo_hbm, bo)]
    cps = [pltpu.make_async_copy(s, d, sems.at[i]) for i, (s, d) in enumerate(pairs)]
    for c in cps[:7]:
        c.start()

    def set_x(p, rows, y):
        xT[p][rows, :] = y

    def run(*gens):
        for _ in zip(*gens):
            pass

    def ln(p):
        for j in range(NJ):
            v = xT[p][:, tile(j)]
            c = v - jnp.mean(v, axis=0, keepdims=True)
            var = jnp.mean(c * c, axis=0, keepdims=True)
            xn[p][:, tile(j)] = _st(c * lax.rsqrt(var + 1e-5))
            yield

    for c in range(NC):
        cps[c].wait()
        if c == 0:
            for cp in cps[7:]:
                cp.start()
        for t in range(2):
            xu[t][...] = pltpu.bitcast(xb[c][:, tile(t)], U32)
            rows = slice(c * GA + t * 128, c * GA + (t + 1) * 128)
            for j in range(NJ):
                v = xu[t][pl.ds(j, 128, stride=NJ), :].T
                xT0[rows, tile(j)] = pltpu.bitcast(v << 16, F32)
                xT1[rows, tile(j)] = pltpu.bitcast(v & jnp.uint32(0xFFFF0000), F32)

    r, cc = _iota((128, 128), 0), _iota((128, 128), 1)
    perm = [jnp.where((r % 4) * DH + ((r // 4) ^ b) == cc, 1.0, 0.0).astype(BF16) for b in range(2)]

    def merge(a, b):
        a, b = a.reshape(16, 8, D), b.reshape(16, 8, D)
        lo = _iota((16, 8, D), 1) < 4
        o = jnp.stack([jnp.where(lo, a, b), pltpu.roll(jnp.where(lo, b, a), 4, 1)], axis=1)
        return o.reshape(GA, D)

    def prep_aq(g):
        for sec in range(3):
            cps[NC + 3 * g + sec].wait()
        for sec in range(3):
            a, b = (_dot_nt(perm[t], aq[g][sec, :, tile(t)]) for t in range(2))
            aqT[g, tile(sec), :] = _st(merge(a, b))

    def prep_ao():
        for cp in cps[-4:]:
            cp.wait()
        for g in range(NC):
            a, b = (_dot(perm[t], ao[tile(2 * g + t), :]) for t in range(2))
            aoT[:, g * GA:(g + 1) * GA] = pltpu.bitcast(merge(a, b).astype(BF16).T, U32)

    def prep_b():
        rep = jnp.where(_iota((DH, GB), 1) % DH == _iota((DH, GB), 0), 1.0, 0.0).astype(BF16)
        for g in range(D // GB):
            bd = jnp.where(r // DH == cc // DH, _dot(phi[tile(g), :], rep), 0.0)
            bdT = bd.T.astype(BF16)
            for sec in range(2):
                bqT[g, sec * 64:(sec + 1) * 64, :] = _st(_dot_nt(bdT, bq[:, tile(sec * 8 + g)]))
            bqT[g, 128:, :] = pltpu.bitcast(bq[:, tile(16 + g)].T, U32)
            boT[:, tile(g)] = pltpu.bitcast(bo[tile(g), :].T, U32)

    def out_proj(wT, p):
        for j in range(NJ):
            xT[p][:, tile(j)] += _dot(_ld(wT[...]), _ld(oT[p][:, tile(j)]))
            yield

    def a_mm(u, slot):
        b, p, g = buf[slot], u // NC, u % NC
        for j in range(NJ):
            y = _dot(_ld(aqT[g]), _ld(xnn[p, :, tile(j)]))
            b[0:3 * GA, tile(j)] = y
            if j:
                b[3 * GA:, tile(j)] = pltpu.roll(y[GA:], 1, 1)
            yield

    def a_att(u, slot):
        b, p, g = buf[slot], u // NC, u % NC
        lane = _iota((8, 128), 1)
        for j in range(NJ):
            def src(sec, w, d):
                sec = sec if j >= w else sec + 2
                return b[pl.ds(sec * GA + d * 8, CD * 8), tile((j - w) % NJ)].reshape(CD, 8, 128)
            lg = [None] * W
            for d in range(0, DH, CD):
                q = src(0, 0, d)
                for w in range(W):
                    l = jnp.sum(q * src(1, w, d), axis=0)
                    lg[w] = l + lg[w] if d else l
            lg = [l * (DH ** -0.5) for l in lg]
            lg = [jnp.where(lane == 0, -1e9, l) if j < w else l for w, l in enumerate(lg)]
            m = functools.reduce(jnp.maximum, lg)
            e = [jnp.exp(l - m) for l in lg]
            inv = 1.0 / sum(e[1:], e[0])
            e = [t * inv for t in e]
            for d in range(0, DH, CD):
                o = e[0] * src(2, 0, d)
                for w in range(1, W):
                    o = o + e[w] * src(2, w, d)
                oTT[p, pl.ds(pl.multiple_of(g * 128 + d * 4, CD * 4), CD * 4), tile(j)] = _st(o.reshape(CD * 8, 128))
            yield

    def layer_a(first):
        n = 2 * NC
        if first:
            prep_aq(0)
            run(ln(0), a_mm(0, 0), ln(1))
            for g in range(1, NC):
                prep_aq(g)
        else:
            run(ln(1), a_mm(0, 0))

        @pl.loop(0, n // 2 - 1)
        def _(i):
            run(a_mm(2 * i + 1, 1), a_att(2 * i, 0))
            run(a_mm(2 * i + 2, 0), a_att(2 * i + 1, 1))

        run(a_mm(n - 1, 1), a_att(n - 2, 0))
        if first:
            prep_ao()
            prep_b()
        run(out_proj(aoT, 0), a_att(n - 1, 1))
        run(out_proj(aoT, 1), ln(0))

    def feat(y):
        outs = []
        for h in range(GB // DH):
            t = y[h * DH:(h + 1) * DH]
            ep = jnp.exp(t - jnp.max(t, axis=0, keepdims=True))
            en = jnp.exp(jnp.min(t, axis=0, keepdims=True) - t)
            outs.append(ep * (1.0 / jnp.sum(ep, axis=0, keepdims=True)))
            outs.append(en * (1.0 / jnp.sum(en, axis=0, keepdims=True)))
        return jnp.concatenate(outs, axis=0)

    def b_qkv(p, g):
        if p == 0 and isinstance(g, int):
            ys = []
            for j, _ in enumerate(ln(1)):
                ys.append(_dot(_ld(bqT[g]), _ld(xn[p][:, tile(j)])))
            y = jnp.concatenate(ys, axis=1)
        else:
            y = _dot(_ld(bqT[g]), _ld(xn[p][...]))
        pq[p][pl.ds(pl.multiple_of(g * 128, 128), 128), :] = _st(feat(y[:GB]))
        fk = feat(y[GB:2 * GB]).astype(BF16)
        ones = jnp.ones((16, HS), BF16)
        for t in range(2):
            v = y[2 * GB + t * 64:2 * GB + (t + 1) * 64].astype(BF16)
            a = _dot_nt(jnp.concatenate([v, ones], axis=0), fk[tile(t)])
            if p == 0:
                kv[2 * g + t] = a
            else:
                rr = _iota((80, 128), 0)
                hd = jnp.where(rr < 64, rr // DH, rr - 64)
                kv[2 * g + t] = jnp.where(hd == _iota((80, 128), 1) // 64, a + kv[2 * g + t], 0.0)

    def b_out(p):
        for t in range(H // 2):
            y = _dot(kv[t].astype(BF16), _ld(pq[p][t * 64:(t + 1) * 64, :]))
            inv = 1.0 / (y[64:72] + 1e-6)
            o = jnp.concatenate([y[h * DH:(h + 1) * DH] * inv[h:h + 1] for h in range(2)], axis=0)
            oT[p][t * DH:(t + 1) * DH, :] = _st(o)
            if t % 2:
                yield

    def finish():
        cps = []
        for c in range(NC):
            rows = slice(c * GA, (c + 1) * GA)
            w = _ld(boT[tile(c), :])
            y0, y1 = (xT[p][rows, :] + _dot(w, _ld(oT[p][...])) for p in range(2))
            u = (_top(y0) >> 16) | _top(y1)
            for t in range(2):
                for j in range(NJ):
                    xu[t][pl.ds(j, 128, stride=NJ), :] = u[tile(t), tile(j)].T
                xb[c][:, tile(t)] = _ld(xu[t][...])
            cps.append(pltpu.make_async_copy(xb[c], out_hbm.at[:, cols(c)], sems.at[c]))
            cps[-1].start()
        for cp in cps:
            cp.wait()

    def layer_b(last):
        for p in range(2):
            if p == 0:
                b_qkv(0, 0)
            pl.loop(1 - p, D // GB)(functools.partial(b_qkv, p))
        run(b_out(0))
        if last:
            run(b_out(1))
            finish()
        else:
            run(out_proj(boT, 0), b_out(1))
            run(out_proj(boT, 1), ln(0))

    for l in range(2):
        layer_a(l == 0)
        layer_b(l == 1)


@jax.jit
def pallas_interleave_layers__sliding_local_dilated__linear_kernel_hedgehog__prompt_kernel(
    A_x, A_wqkv, A_wo, B_x, B_wqkv, B_w_phi, B_wo,
):
    del B_x
    vm = pltpu.VMEM
    out = pl.pallas_call(
        _kernel,
        out_shape=jax.ShapeDtypeStruct((S, D), BF16),
        in_specs=[pl.BlockSpec(memory_space=pl.ANY)] * 6,
        out_specs=pl.BlockSpec(memory_space=pl.ANY),
        scratch_shapes=[
            *[vm((S, GA), BF16)] * 4, *[vm((HS, 128), U32)] * 2, *[vm((3, D, GA), BF16)] * 4,
            vm((D, D), BF16), vm((D, 3 * D), BF16), vm((D, D), BF16), vm((D, DH), BF16),
            vm((D // GA, 3 * GA // 2, D), U32), vm((D // 2, D), U32),
            vm((D // GB, 3 * GB // 2, D), U32), vm((D // 2, D), U32),
            *[vm((D, HS), F32)] * 2, *[vm((2, D // 2, HS), U32)] * 2,
            *[vm((5 * GA, HS), F32)] * 2, *[vm((D, HS), U32)] * 2,
            vm((H // 2, 80, 128), F32),
            pltpu.SemaphoreType.DMA((20,)),
        ],
        compiler_params=pltpu.CompilerParams(vmem_limit_bytes=120 * 1024 * 1024),
    )(A_x.reshape(S, D), A_wqkv, A_wo, B_wqkv, B_w_phi.reshape(D, DH), B_wo)
    return out.reshape(1, S, D)
```
